```python
import os as _os
_os.environ.setdefault("JAX_PLATFORMS", "cpu")
import jax
import jax.numpy as jnp

def _softmax(x, axis=-1):
    return jax.nn.softmax(x, axis=axis)
def _gelu(x):
    return jax.nn.gelu(x, approximate=True)
def _silu(x):
    return jax.nn.silu(x)
def _sigmoid(x):
    return jax.nn.sigmoid(x)
def _layernorm(x, axis=-1, eps=1e-5):
    m = jnp.mean(x, axis=axis, keepdims=True)
    v = jnp.var(x, axis=axis, keepdims=True)
    return (x - m) / jnp.sqrt(v + eps)
def _scatter_add(tgt, idx, src, axis=0):
    return tgt.at[idx].add(src)
def _segment_sum(src, seg, n):
    return jax.ops.segment_sum(src, seg, n)
class _Rng:
    def __init__(self, key):
        self._k = key
    def _next(self):
        self._k, sub = jax.random.split(self._k)
        return sub
    def normal(self, shape):
        return jax.random.normal(self._next(), shape, dtype=jnp.bfloat16)
    def randint(self, lo, hi, shape):
        return jax.random.randint(self._next(), shape, lo, hi, dtype=jnp.int32)
    def uniform(self, shape, lo=0.0, hi=1.0):
        return jax.random.uniform(self._next(), shape, jnp.bfloat16, lo, hi)
    def permutation(self, n):
        return jax.random.permutation(self._next(), n)


kernel_name = 'gated_mix__linear_kernel_hedgehog__glu_gated_bilinear__prompt'

def setup_inputs():
    _rng = _Rng(jax.random.key(int.from_bytes(__import__("os").urandom(4), "little")))
    _w = (lambda a: (lambda t: t.astype(jnp.bfloat16) if jnp.issubdtype(t.dtype, jnp.floating) else t)(jnp.asarray(a)))
    def _A_setup():
        B, S, D, H = 1, 2048, 512, 32
        Dh = D // H
        return {
            "x": _w((lambda *s: _rng.normal(s) * 0.05)(B, S, D)),
            "wqkv": _w((lambda *s: _rng.normal(s) * 0.8)(D, 3 * D)),
            "w_phi": _w((lambda *s: _rng.normal(s) * 0.8)(H, Dh, Dh) * (Dh ** -0.5)),
            "wo": _w((lambda *s: _rng.normal(s) * 0.05)(D, D)),
        }
    _A_in = _A_setup()

    def _B_setup():
        B, S, D, F = 1, 2048, 512, 1792
        return {
            "x": _w((lambda *s: _rng.normal(s) * 0.05)(B, S, D)),
            "w_gate": _w((lambda *s: _rng.normal(s) * 1.6)(D, F) * (D ** -0.5)),
            "w_up": _w((lambda *s: _rng.normal(s) * 1.6)(D, F) * (D ** -0.5)),
            "w_down": _w((lambda *s: _rng.normal(s) * 1.6)(F, D) * (F ** -0.5)),
        }
    _B_in = _B_setup()

    return {
        "A_x": _A_in["x"],
        "A_wqkv": _A_in["wqkv"],
        "A_w_phi": _A_in["w_phi"],
        "A_wo": _A_in["wo"],
        "B_x": _B_in["x"],
        "B_w_gate": _B_in["w_gate"],
        "B_w_up": _B_in["w_up"],
        "B_w_down": _B_in["w_down"],
        "gate_w": _w((lambda *s: _rng.normal(s) * 0.05)(512) * 16.0),
    }

def reference(A_x, A_wqkv, A_w_phi, A_wo, B_x, B_w_gate, B_w_up, B_w_down, gate_w):
    def _A_ref(x, wqkv, w_phi, wo):
        B, S, D = x.shape
        H = 32; Dh = D // H
        qkv = (lambda x, *d: x.transpose(*d))((x @ wqkv).reshape(B, S, 3, H, Dh), 2, 0, 3, 1, 4)
        q, k, v = qkv[0], qkv[1], qkv[2]
        pq = jnp.einsum("bhsd,hdf->bhsf", q, w_phi)
        pk = jnp.einsum("bhsd,hdf->bhsf", k, w_phi)
        phi_q = jnp.concatenate([_softmax(pq, axis=-1), _softmax(-pq, axis=-1)], axis=-1)
        phi_k = jnp.concatenate([_softmax(pk, axis=-1), _softmax(-pk, axis=-1)], axis=-1)
        kv = jnp.einsum("bhsf,bhsd->bhfd", phi_k, v)
        z  = jnp.einsum("bhsf->bhf", phi_k)
        num = jnp.einsum("bhqf,bhfd->bhqd", phi_q, kv)
        den = jnp.einsum("bhqf,bhf->bhq", phi_q, z)[..., None] + 1e-6
        o = num / den
        return (lambda x, *d: x.transpose(*d))(o, 0, 2, 1, 3).reshape(B, S, D) @ wo

    def _B_ref(x, w_gate, w_up, w_down):
        g = jnp.einsum("bsd,df->bsf", x, w_gate)
        u = jnp.einsum("bsd,df->bsf", x, w_up)
        h = g * u
        return jnp.einsum("bsf,fd->bsd", h, w_down)

    x = A_x
    g = _sigmoid((x * gate_w).sum(-1, keepdims=True))
    a = _A_ref(x, A_wqkv, A_w_phi, A_wo)
    b = _B_ref(x, B_w_gate, B_w_up, B_w_down)
    return g * a + (1 - g) * b
```

```python
import jax
import jax.numpy as jnp
from jax import lax
import jax.experimental.pallas as pl
import jax.experimental.pallas.tpu as pltpu

S, D, H, DH, F = 2048, 512, 32, 16, 1792
G = D // 128
TM1 = 512
TM2 = 512
UNROLL1 = False
UNROLL2 = False
f32, bf16 = jnp.float32, jnp.bfloat16

NT_DIMS = (((1,), (1,)), ((), ()))


def _dot(a, b):
    return jnp.dot(a, b, preferred_element_type=f32)


def _dot_nt(a, b):
    return lax.dot_general(a, b, NT_DIMS, preferred_element_type=f32)


def _iota(shape, dim):
    return lax.broadcasted_iota(jnp.int32, shape, dim)


def _dual_softmax_t(p):
    t = p.shape[1]
    p3 = p.reshape(16, 8, t)
    mx = jnp.max(p3, axis=0, keepdims=True)
    mn = jnp.min(p3, axis=0, keepdims=True)
    ep = jnp.exp(p3 - mx)
    en = jnp.exp(mn - p3)
    rp = 1.0 / jnp.sum(ep, axis=0, keepdims=True)
    rn = 1.0 / jnp.sum(en, axis=0, keepdims=True)
    return (ep * rp).reshape(128, t), (en * rn).reshape(128, t)


def kernel(x_hbm, wqkv_hbm, wphi_ref, wo_hbm, wg_hbm, wu_hbm, wd_hbm, gw_ref, o_hbm,
           x_ref, wqkv_ref, wo_ref, wg_ref, wu_ref, wd_ref, o_ref,
           wt_ref, kv_ref, z_ref, m_ref, xsem, wsem, osem):
    n1 = S // TM1
    n2 = S // TM2

    def x_copy(i):
        return pltpu.make_async_copy(x_hbm.at[pl.ds(i * TM1, TM1), :], x_ref.at[pl.ds(i * TM1, TM1), :], xsem.at[i])

    def o_copy(i):
        return pltpu.make_async_copy(o_ref.at[pl.ds(i * TM2, TM2), :], o_hbm.at[pl.ds(i * TM2, TM2), :], osem.at[i])

    def qkv_copy(j):
        return pltpu.make_async_copy(wqkv_hbm.at[:, pl.ds(j * D, D)], wqkv_ref.at[:, pl.ds(j * D, D)], wsem.at[j])

    w_copies = [pltpu.make_async_copy(a, b, wsem.at[3 + n]) for n, (a, b) in enumerate(
        [(wg_hbm, wg_ref), (wu_hbm, wu_ref), (wd_hbm, wd_ref), (wo_hbm, wo_ref)])]

    qkv_copy(1).start()
    qkv_copy(2).start()
    x_copy(0).start()
    for i in range(1, n1):
        x_copy(i).start()
    qkv_copy(0).start()
    for c in w_copies:
        c.start()

    sel = jnp.where(_iota((H, D), 0) == _iota((H, D), 1) // DH, 1.0, 0.0).astype(bf16)
    a = _dot(wphi_ref[...], sel)
    a = jnp.where(_iota((256, D), 0) // DH == _iota((256, D), 1) % DH, a, 0.0).astype(bf16)
    lsel = jnp.where(_iota((128, 256), 0) // 8 == _iota((128, 256), 1) % DH, 1.0, 0.0).astype(bf16)
    phit = _dot(lsel, a)
    phit = jnp.where(_iota((128, D), 0) % 8 == (_iota((128, D), 1) // DH) % 8, phit, 0.0).astype(bf16)

    def fold(j):
        for g in range(G):
            w = wqkv_ref[:, j * D + g * 128: j * D + (g + 1) * 128]
            wt_ref[j * D + g * 128: j * D + (g + 1) * 128, :] = _dot_nt(phit[:, g * 128:(g + 1) * 128], w).astype(bf16)

    kv_ref[...] = jnp.zeros_like(kv_ref)
    z_ref[...] = jnp.zeros_like(z_ref)
    qkv_copy(1).wait()
    fold(1)
    qkv_copy(2).wait()
    wt_ref[2 * D:3 * D, :] = wqkv_ref[:, 2 * D:3 * D].T

    def phase1(i, carry):
        x_copy(i).wait()
        x = x_ref[pl.ds(pl.multiple_of(i * TM1, TM1), TM1), :]
        kvt = _dot_nt(wt_ref[D:3 * D, :], x)
        for g in range(G):
            pp, pn = _dual_softmax_t(kvt[g * 128:(g + 1) * 128, :])
            phi = jnp.concatenate([pp, pn], axis=0)
            vt = kvt[D + g * 128: D + (g + 1) * 128, :].astype(bf16)
            kv_ref[g] += _dot_nt(vt, phi.astype(bf16))
            zz = phi[:, 0:128]
            for c in range(1, TM1 // 128):
                zz = zz + phi[:, c * 128:(c + 1) * 128]
            z_ref[g] += zz
        return carry

    if UNROLL1:
        for i in range(n1):
            phase1(i, 0)
    else:
        lax.fori_loop(0, n1, phase1, 0)

    qkv_copy(0).wait()
    fold(0)
    msk = _iota((128, 256), 0) // 16 == _iota((128, 256), 1) % 8
    msk2 = _iota((16, 256), 0) == _iota((16, 256), 1) % 8
    for g in range(G):
        m_ref[g, 0:128, :] = jnp.where(msk, kv_ref[g], 0.0).astype(bf16)
        zrow = jnp.sum(z_ref[g].T, axis=0, keepdims=True)
        m_ref[g, 128:144, :] = jnp.where(msk2, zrow, 0.0).astype(bf16)
    for c in w_copies:
        c.wait()

    def phase2(i, carry):
        rows = pl.ds(pl.multiple_of(i * TM2, TM2), TM2)
        x = x_ref[rows, :]
        qt = _dot_nt(wt_ref[0:D, :], x)
        os_ = []
        for g in range(G):
            pp, pn = _dual_softmax_t(qt[g * 128:(g + 1) * 128, :])
            phi = jnp.concatenate([pp, pn], axis=0).astype(bf16)
            nd = _dot(m_ref[g], phi)
            rd = 1.0 / (nd[128:136, :] + 1e-6)
            num = nd[0:128, :].reshape(8, 16, TM2)
            o = num * rd.reshape(8, 1, TM2)
            os_.append(o.reshape(128, TM2))
        ot = jnp.concatenate(os_, axis=0).astype(bf16)
        a = _dot(ot.T, wo_ref[...])
        gg = _dot(x, wg_ref[...])
        uu = _dot(x, wu_ref[...])
        b = _dot((gg * uu).astype(bf16), wd_ref[...])
        gate = jax.nn.sigmoid(jnp.sum(x.astype(f32) * gw_ref[...].astype(f32)[None, :], axis=-1, keepdims=True))
        o_ref[rows, :] = (gate * a + (1.0 - gate) * b).astype(bf16)
        o_copy(i).start()
        return carry

    if UNROLL2:
        for i in range(n2):
            phase2(i, 0)
    else:
        lax.fori_loop(0, n2, phase2, 0)
    for i in range(n2):
        o_copy(i).wait()


@jax.jit
def pallas_gated_mix__linear_kernel_hedgehog__glu_gated_bilinear__prompt_kernel(
    A_x, A_wqkv, A_w_phi, A_wo, B_x, B_w_gate, B_w_up, B_w_down, gate_w):
    x = A_x.reshape(S, D)
    hbm = pl.BlockSpec(memory_space=pl.ANY)
    vmem = pl.BlockSpec(memory_space=pltpu.VMEM)
    out = pl.pallas_call(
        kernel,
        in_specs=[hbm, hbm, vmem, hbm, hbm, hbm, hbm, vmem],
        out_specs=hbm,
        out_shape=jax.ShapeDtypeStruct((S, D), bf16),
        scratch_shapes=[
            pltpu.VMEM((S, D), bf16),
            pltpu.VMEM((D, 3 * D), bf16),
            pltpu.VMEM((D, D), bf16),
            pltpu.VMEM((D, F), bf16),
            pltpu.VMEM((D, F), bf16),
            pltpu.VMEM((F, D), bf16),
            pltpu.VMEM((S, D), bf16),
            pltpu.VMEM((3 * D, D), bf16),
            pltpu.VMEM((G, 128, 256), f32),
            pltpu.VMEM((G, 256, 128), f32),
            pltpu.VMEM((G, 144, 256), bf16),
            pltpu.SemaphoreType.DMA((S // TM1,)),
            pltpu.SemaphoreType.DMA((7,)),
            pltpu.SemaphoreType.DMA((S // TM2,)),
        ],
        compiler_params=pltpu.CompilerParams(
            vmem_limit_bytes=100 * 1024 * 1024),
    )(x, A_wqkv, A_w_phi.transpose(1, 2, 0).reshape(DH * DH, H), A_wo, B_w_gate, B_w_up, B_w_down, gate_w)
    return out.reshape(1, S, D)
```

```python
import jax
import jax.numpy as jnp
from jax import lax
import jax.experimental.pallas as pl
import jax.experimental.pallas.tpu as pltpu

S, D, H, DH, F = 2048, 512, 32, 16, 1792
G = D // 128
TM1 = 512
TM2 = 512
f32, bf16 = jnp.float32, jnp.bfloat16

NT_DIMS = (((1,), (1,)), ((), ()))


def _dot(a, b):
    return jnp.dot(a, b, preferred_element_type=f32)


def _dot_nt(a, b):
    return lax.dot_general(a, b, NT_DIMS, preferred_element_type=f32)


def _iota(shape, dim):
    return lax.broadcasted_iota(jnp.int32, shape, dim)


def _dual_softmax_t(p):
    t = p.shape[1]
    p3 = p.reshape(16, 8, t)
    r3 = -pltpu.roll(p3, 4, 1)
    lo = _iota((16, 8, t), 1) < 4
    out = []
    for a in (jnp.where(lo, p3, r3), jnp.where(lo, r3, p3)):
        e = jnp.exp(a - jnp.max(a, axis=0, keepdims=True))
        out.append(e * (1.0 / jnp.sum(e, axis=0, keepdims=True)))
    return out


def _quads(a, r, c):
    return a[:r, :c], a[:r, c:], a[r:, :c], a[r:, c:]


def _lhs7(a11, a12, a21, a22):
    return [a11 + a22, a21 + a22, a11, a22, a11 + a12, a21 - a11, a12 - a22]


def _comb7(m):
    return m[0] + m[3] - m[4] + m[6], m[2] + m[4], m[1] + m[3], m[0] - m[1] + m[2] + m[5]


def _rhs(w_ref, s_ref, n, first):
    r, c = w_ref.shape[0] // 2, w_ref.shape[1] // 2
    if n == 1:
        return w_ref[:r, :c]
    if n == 4:
        return w_ref[r:, c:]
    k = {0: 0, 2: 1, 3: 2, 5: 3, 6: 4}[n]
    if not first:
        return s_ref[k]
    b11, b12, b21, b22 = _quads(w_ref[...].astype(f32), r, c)
    t = (b11 + b22, b12 - b22, b21 - b11, b11 + b12, b21 + b22)[k].astype(bf16)
    s_ref[k] = t
    return t


def kernel(x_hbm, wqkv_hbm, wphi_ref, wo_hbm, wg_hbm, wu_hbm, wd_hbm, gw_ref, o_hbm,
           x_ref, wqkv_ref, wo_ref, wg_ref, wu_ref, wd_ref, o_ref,
           wt_ref, kv_ref, z_ref, m_ref, sg_ref, su_ref, sd_ref, xsem, wsem, osem):
    n1 = S // TM1
    n2 = S // TM2

    def x_copy(i):
        return pltpu.make_async_copy(x_hbm.at[pl.ds(i * TM1, TM1), :], x_ref.at[pl.ds(i * TM1, TM1), :], xsem.at[i])

    def o_copy(i):
        return pltpu.make_async_copy(o_ref.at[pl.ds(i * TM2, TM2), :], o_hbm.at[pl.ds(i * TM2, TM2), :], osem.at[i])

    def qkv_copy(j):
        return pltpu.make_async_copy(wqkv_hbm.at[:, pl.ds(j * D, D)], wqkv_ref.at[:, pl.ds(j * D, D)], wsem.at[j])

    w_copies = [pltpu.make_async_copy(a, b, wsem.at[3 + n]) for n, (a, b) in enumerate(
        [(wg_hbm, wg_ref), (wu_hbm, wu_ref), (wd_hbm, wd_ref), (wo_hbm, wo_ref)])]

    qkv_copy(1).start()
    qkv_copy(2).start()
    x_copy(0).start()

    sel = jnp.where(_iota((H, D), 0) == _iota((H, D), 1) // DH, 1.0, 0.0).astype(bf16)
    a = _dot(wphi_ref[...], sel)
    a = jnp.where(_iota((256, D), 0) // DH == _iota((256, D), 1) % DH, a, 0.0).astype(bf16)
    lsel = jnp.where(_iota((128, 256), 0) // 8 == _iota((128, 256), 1) % DH, 1.0, 0.0).astype(bf16)
    phit = _dot(lsel, a)
    phit = jnp.where(_iota((128, D), 0) % 8 == (_iota((128, D), 1) // DH) % 8, phit, 0.0).astype(bf16)

    def fold(j):
        for g in range(G):
            w = wqkv_ref[:, j * D + g * 128: j * D + (g + 1) * 128]
            wt_ref[j * D + g * 128: j * D + (g + 1) * 128, :] = _dot_nt(phit[:, g * 128:(g + 1) * 128], w).astype(bf16)

    qkv_copy(1).wait()
    qkv_copy(2).wait()
    x_copy(1).start()
    w_copies[0].start()
    fold(1)
    wt_ref[2 * D:3 * D, :] = wqkv_ref[:, 2 * D:3 * D].T

    kv_ref[...] = jnp.zeros_like(kv_ref)
    z_ref[...] = jnp.zeros_like(z_ref)

    def phase1(i, carry):
        x_copy(i).wait()
        for n in range(1, n1):
            @pl.when(i == n)
            def _():
                w_copies[n - 1].wait()
                if n + 1 < n1:
                    x_copy(n + 1).start()
                w_copies[n].start()
                if n == n1 - 1:
                    qkv_copy(0).start()
        x = x_ref[pl.ds(pl.multiple_of(i * TM1, TM1), TM1), :]
        kt = _dot_nt(wt_ref[D:2 * D, :], x)
        vt = _dot_nt(wt_ref[2 * D:3 * D, :], x).astype(bf16)
        for g in range(G):
            for j, phi in enumerate(_dual_softmax_t(kt[g * 128:(g + 1) * 128, :])):
                q = 2 * g + j
                phi = phi.reshape(128, TM1)
                kv = _dot_nt(vt[q * 64:(q + 1) * 64, :], phi.astype(bf16))
                zz = phi[:, 0:128]
                for c in range(1, TM1 // 128):
                    zz = zz + phi[:, c * 128:(c + 1) * 128]
                kv_ref[q] += kv
                z_ref[q] += zz
        return carry

    lax.fori_loop(0, n1, phase1, 0)
    qkv_copy(0).wait()
    w_copies[3].wait()
    fold(0)
    msk = _iota((64, 128), 0) // 16 == _iota((64, 128), 1) % 4
    for q in range(2 * G):
        m_ref[q] = jnp.where(msk, kv_ref[q], 0.0).astype(bf16)
        z_ref[q] = jnp.broadcast_to(jnp.sum(z_ref[q], axis=1, keepdims=True), (128, 128))

    def phase2(i, carry, first=False):
        rows = pl.ds(0 if first else pl.multiple_of(i * TM2, TM2), TM2)
        x = x_ref[rows, :]
        qt = _dot_nt(wt_ref[0:D, :], x)
        xf = x.astype(f32)
        xs = [t.astype(bf16) for t in _lhs7(*_quads(xf, TM2 // 2, D // 2))]
        gate = jax.nn.sigmoid(jnp.sum(xf * gw_ref[...].astype(f32)[None, :], axis=-1, keepdims=True))
        jobs = [(wg_ref, sg_ref, n) for n in range(7)] + [(wu_ref, su_ref, n) for n in range(7)]
        ms = []
        os_ = []
        for g in range(G):
            for j, phi in enumerate(_dual_softmax_t(qt[g * 128:(g + 1) * 128, :])):
                q = 2 * g + j
                for w_ref, s_ref, n in jobs[len(ms):len(ms) + (2 if q < 6 else 1)]:
                    ms.append(_dot(xs[n], _rhs(w_ref, s_ref, n, first)))
                num = _dot(m_ref[q], phi.reshape(128, TM2).astype(bf16))
                zb = jnp.concatenate([z_ref[q]] * (TM2 // 128), axis=1).reshape(16, 8, TM2)
                w = jnp.sum(phi * zb, axis=0)
                rd = 1.0 / (w + pltpu.roll(w, 4, 0) + 1e-6)
                o = num.reshape(4, 16, TM2) * rd[0:4].reshape(4, 1, TM2)
                os_.append(o.reshape(64, TM2))
        ot = jnp.concatenate(os_, axis=0).astype(bf16)
        a = gate * _dot(ot.T, wo_ref[...])
        gq = _comb7(ms[:7])
        uq = _comb7(ms[7:])
        hs = [t.astype(bf16) for t in _lhs7(*[p * q for p, q in zip(gq, uq)])]
        b11, b12, b21, b22 = _comb7([_dot(hs[n], _rhs(wd_ref, sd_ref, n, first)) for n in range(7)])
        b = jnp.concatenate([jnp.concatenate([b11, b12], axis=1), jnp.concatenate([b21, b22], axis=1)], axis=0)
        o_ref[rows, :] = (a + (1.0 - gate) * b).astype(bf16)
        o_copy(i).start()
        return carry

    phase2(0, 0, True)
    lax.fori_loop(1, n2, phase2, 0)
    for i in range(n2):
        o_copy(i).wait()


@jax.jit
def pallas_gated_mix__linear_kernel_hedgehog__glu_gated_bilinear__prompt_kernel(
    A_x, A_wqkv, A_w_phi, A_wo, B_x, B_w_gate, B_w_up, B_w_down, gate_w):
    del B_x
    x = A_x.reshape(S, D)
    hbm = pl.BlockSpec(memory_space=pl.ANY)
    vmem = pl.BlockSpec(memory_space=pltpu.VMEM)
    out = pl.pallas_call(
        kernel,
        in_specs=[hbm, hbm, vmem, hbm, hbm, hbm, hbm, vmem],
        out_specs=hbm,
        out_shape=jax.ShapeDtypeStruct((S, D), bf16),
        scratch_shapes=[
            pltpu.VMEM((S, D), bf16),
            pltpu.VMEM((D, 3 * D), bf16),
            pltpu.VMEM((D, D), bf16),
            pltpu.VMEM((D, F), bf16),
            pltpu.VMEM((D, F), bf16),
            pltpu.VMEM((F, D), bf16),
            pltpu.VMEM((S, D), bf16),
            pltpu.VMEM((3 * D, D), bf16),
            pltpu.VMEM((2 * G, 64, 128), f32),
            pltpu.VMEM((2 * G, 128, 128), f32),
            pltpu.VMEM((2 * G, 64, 128), bf16),
            pltpu.VMEM((5, D // 2, F // 2), bf16),
            pltpu.VMEM((5, D // 2, F // 2), bf16),
            pltpu.VMEM((5, F // 2, D // 2), bf16),
            pltpu.SemaphoreType.DMA((S // TM1,)),
            pltpu.SemaphoreType.DMA((7,)),
            pltpu.SemaphoreType.DMA((S // TM2,)),
        ],
        compiler_params=pltpu.CompilerParams(
            vmem_limit_bytes=100 * 1024 * 1024),
    )(x, A_wqkv, A_w_phi.transpose(1, 2, 0).reshape(DH * DH, H), A_wo, B_w_gate, B_w_up, B_w_down, gate_w)
    return out.reshape(1, S, D)
```
